```python
import os as _os
_os.environ.setdefault("JAX_PLATFORMS", "cpu")
import jax
import jax.numpy as jnp

def _softmax(x, axis=-1):
    return jax.nn.softmax(x, axis=axis)
def _gelu(x):
    return jax.nn.gelu(x, approximate=True)
def _silu(x):
    return jax.nn.silu(x)
def _sigmoid(x):
    return jax.nn.sigmoid(x)
def _layernorm(x, axis=-1, eps=1e-5):
    m = jnp.mean(x, axis=axis, keepdims=True)
    v = jnp.var(x, axis=axis, keepdims=True)
    return (x - m) / jnp.sqrt(v + eps)
def _scatter_add(tgt, idx, src, axis=0):
    return tgt.at[idx].add(src)
def _segment_sum(src, seg, n):
    return jax.ops.segment_sum(src, seg, n)
class _Rng:
    def __init__(self, key):
        self._k = key
    def _next(self):
        self._k, sub = jax.random.split(self._k)
        return sub
    def normal(self, shape):
        return jax.random.normal(self._next(), shape, dtype=jnp.bfloat16)
    def randint(self, lo, hi, shape):
        return jax.random.randint(self._next(), shape, lo, hi, dtype=jnp.int32)
    def uniform(self, shape, lo=0.0, hi=1.0):
        return jax.random.uniform(self._next(), shape, jnp.bfloat16, lo, hi)
    def permutation(self, n):
        return jax.random.permutation(self._next(), n)


kernel_name = 'standalone__detection_seg_fpn_lateral__vision'

def setup_inputs():
    _rng = _Rng(jax.random.key(int.from_bytes(__import__("os").urandom(4), "little")))
    _w = (lambda a: (lambda t: t.astype(jnp.bfloat16) if jnp.issubdtype(t.dtype, jnp.floating) else t)(jnp.asarray(a)))
    H = W = (256 // 2) * 2
    C = 384
    k = 1
    return {
        "c_fine": _w((lambda *s: _rng.normal(s) * 0.05)(1, H, W, C)),
        "p_coarse": _w((lambda *s: _rng.normal(s) * 0.05)(1, H // 2, W // 2, C)),
        "w_lat": _w((lambda *s: _rng.normal(s) * 0.05)(C, C)),
        "w_out": _w((lambda *s: _rng.normal(s) * 0.05)(k, k, C, C)),
    }

def reference(c_fine, p_coarse, w_lat, w_out):
    B, H, W, C = c_fine.shape
    k = 1
    lat = jnp.einsum("bhwc,cd->bhwd", c_fine, w_lat)
    up = jnp.repeat(jnp.repeat(p_coarse, 2, axis=1), 2, axis=2)
    m = lat + up
    pad = k // 2
    mp = jnp.pad(m, ((0, 0), (pad, pad), (pad, pad), (0, 0)))
    o = None
    for di in range(k):
        for dj in range(k):
            t = jnp.einsum("bhwc,cd->bhwd", mp[:, di:di + H, dj:dj + W, :], w_out[di, dj])
            o = t if o is None else o + t
    return o
```

```python
import jax
import jax.numpy as jnp
from jax import lax
import jax.experimental.pallas as pl
import jax.experimental.pallas.tpu as pltpu

_LANES = 128
_BANDS = 8
_ROWS_PER_STEP = 2
_WRITE_PIXELS = 64
_READ_BOUNDS = (0, 1, 2, 4, 7, 11, 16)
_SWITCH_STEP = 37
_WRITE_BURST = 11
_WRITES_PER_STEP = 5


def _upsample_rows(q):
    n, ch = q.shape
    tiles = []
    for lo in range(0, ch, _LANES):
        t = q[:, lo:lo + _LANES]
        tiles.append(jnp.concatenate([t, t], axis=1).reshape(2 * n, _LANES))
    return jnp.concatenate(tiles, axis=1)


def _fpn_kernel(c_hbm, p_hbm, wl_hbm, wo_hbm, o_hbm,
                c_buf, p_buf, o_buf, wl_buf, wo_buf, wf_buf, read_sem, write_sem):
    bands, rows, _, width, ch = c_buf.shape
    u = _ROWS_PER_STEP
    m = _WRITE_PIXELS
    steps_per_row = bands // u
    writes_per_row = 2 * (width // m)
    n_groups = len(_READ_BOUNDS) - 1

    def read(src, dst, idx, k):
        return pltpu.make_async_copy(src.at[idx], dst.at[idx], read_sem.at[k])

    weights = [
        pltpu.make_async_copy(wl_hbm, wl_buf, read_sem.at[n_groups + 1]),
        pltpu.make_async_copy(wo_hbm, wo_buf, read_sem.at[n_groups + 1]),
    ]
    groups, wait_step = [], []
    for k in range(n_groups - 1):
        lo, hi = _READ_BOUNDS[k], _READ_BOUNDS[k + 1]
        idx = (slice(None), pl.ds(lo, hi - lo))
        groups.append([read(p_hbm, p_buf, idx, k), read(c_hbm, c_buf, idx, k)])
        wait_step.append(lo * steps_per_row)
    k = n_groups - 1
    lo, hi = _READ_BOUNDS[k], _READ_BOUNDS[k + 1]
    groups.append([
        read(p_hbm, p_buf, (slice(None), pl.ds(lo, hi - lo)), k),
        read(c_hbm, c_buf, (slice(None), pl.ds(lo, hi - lo - 1)), k),
        read(c_hbm, c_buf, (pl.ds(0, bands - 1), pl.ds(hi - 1, 1)), k),
    ])
    groups.append([read(c_hbm, c_buf, (pl.ds(bands - 1, 1), pl.ds(hi - 1, 1)), k + 1)])
    wait_step += [_SWITCH_STEP, _SWITCH_STEP + 1]
    assert hi == rows and _SWITCH_STEP + 1 <= lo * steps_per_row

    for copy in weights:
        copy.start()
    for group in groups:
        for copy in group:
            copy.start()

    for copy in weights:
        copy.wait()
    wf_buf[...] = jnp.dot(
        wl_buf[...], wo_buf[...], preferred_element_type=jnp.float32
    ).astype(wf_buf.dtype)

    def write(d, carry):
        row, r = d // writes_per_row, d % writes_per_row
        px = pl.ds(pl.multiple_of((r % (width // m)) * m, m), m)
        idx = (slice(None), row, r // (width // m), px)
        pltpu.make_async_copy(o_buf.at[idx], o_hbm.at[idx], write_sem).start()
        return carry

    def step(i, written):
        for group, at in zip(groups, wait_step):
            @pl.when(i == at)
            def _(group=group):
                for copy in group:
                    copy.wait()

        row = i // steps_per_row
        target = jnp.where(
            i >= _SWITCH_STEP,
            jnp.minimum(row * writes_per_row,
                        _WRITE_BURST + _WRITES_PER_STEP * (i - _SWITCH_STEP)),
            0,
        )
        lax.fori_loop(written, target, write, None)

        band = (i % steps_per_row) * u
        coarse = p_buf[pl.ds(band, u), row].reshape(u * (width // 2), ch)
        top = jnp.dot(coarse, wo_buf[...], preferred_element_type=jnp.float32)
        top = _upsample_rows(top).reshape(u, 1, width, ch)
        for s in range(u):
            fine = c_buf[band + s, row].reshape(2 * width, ch)
            lat = jnp.dot(fine, wf_buf[...], preferred_element_type=jnp.float32)
            o_buf[band + s, row] = (lat.reshape(2, width, ch) + top[s]).astype(o_buf.dtype)
        return target

    written = lax.fori_loop(0, rows * steps_per_row, step, jnp.int32(0))
    lax.fori_loop(written, rows * writes_per_row, write, None)
    pltpu.make_async_copy(o_buf, o_hbm, write_sem).wait()


@jax.jit
def pallas_standalone__detection_seg_fpn_lateral__vision_kernel(
    c_fine: jax.Array,
    p_coarse: jax.Array,
    w_lat: jax.Array,
    w_out: jax.Array,
):
    batch, height, width, ch = c_fine.shape
    dtype = c_fine.dtype
    rows = batch * height // 2 // _BANDS
    fine_shape = (_BANDS, rows, 2, width, ch)
    coarse_shape = (_BANDS, rows, width // 2, ch)

    out = pl.pallas_call(
        _fpn_kernel,
        in_specs=[pl.BlockSpec(memory_space=pltpu.HBM)] * 4,
        out_specs=pl.BlockSpec(memory_space=pltpu.HBM),
        out_shape=jax.ShapeDtypeStruct(fine_shape, dtype),
        scratch_shapes=[
            pltpu.VMEM(fine_shape, dtype),
            pltpu.VMEM(coarse_shape, dtype),
            pltpu.VMEM(fine_shape, dtype),
            pltpu.VMEM((ch, ch), dtype),
            pltpu.VMEM((ch, ch), dtype),
            pltpu.VMEM((ch, ch), dtype),
            pltpu.SemaphoreType.DMA((len(_READ_BOUNDS) + 1,)),
            pltpu.SemaphoreType.DMA(()),
        ],
        compiler_params=pltpu.CompilerParams(vmem_limit_bytes=126 * 2**20),
    )(
        c_fine.reshape(fine_shape),
        p_coarse.reshape(coarse_shape),
        w_lat,
        w_out.reshape(ch, ch),
    )
    return out.reshape(batch, height, width, ch)
```

```python
import functools

import jax
import jax.numpy as jnp
from jax import lax
import jax.experimental.pallas as pl
import jax.experimental.pallas.tpu as pltpu

_LANES = 128
_TILE = 16
_HALVES = 2
_STREAMS = 3
_RUN = 48
_READ_GROUPS = (0, 1, 2, 4, 7, 12)
_READ_TAIL = 256
_SWITCH_STEP = 36
_ROUNDS_AT_SWITCH = 12
_ROUNDS_PER_STEP = 7


def _upsample_rows(q):
    n, ch = q.shape
    tiles = []
    for lo in range(0, ch, _LANES):
        t = q[:, lo:lo + _LANES]
        tiles.append(jnp.concatenate([t, t], axis=1).reshape(2 * n, _LANES))
    return jnp.concatenate(tiles, axis=1)


def _fpn_kernel(c_hbm, p_hbm, wl_hbm, wo_hbm, o_hbm,
                c_buf, p_buf, o_buf, wl_buf, wo_buf, wf_buf, write_sem, *, width):
    _, pixels, ch = c_buf.shape
    fine = 2 * width
    coarse = width // 2
    steps = pixels // fine
    span = steps // _STREAMS

    def unit_of(step):
        return (_STREAMS - 1 - step % _STREAMS) * span + step // _STREAMS

    unit_edges = [s * span for s in range(_STREAMS)] + [steps]
    stride = -(-pixels // (_STREAMS * _TILE)) * _TILE
    write_edges = [s * stride for s in range(_STREAMS)] + [pixels]
    rounds = (pixels - write_edges[-2]) // _RUN

    def rounds_queued(step):
        return _ROUNDS_AT_SWITCH + _ROUNDS_PER_STEP * (step - _SWITCH_STEP)

    assert sorted(unit_of(i) for i in range(steps)) == list(range(steps))
    assert _STREAMS * _READ_GROUPS[-2] < _SWITCH_STEP <= _STREAMS * _READ_GROUPS[-1]
    assert rounds_queued(steps) <= rounds
    for i in range(_SWITCH_STEP, steps):
        finished = [unit_of(j) for j in range(i)]
        for lo in write_edges[:-1]:
            hi = lo + rounds_queued(i + 1) * _RUN
            assert all(u in finished for u in range(lo // fine, (hi - 1) // fine + 1))

    def write(start, size):
        idx = (slice(None), pl.ds(start, size))
        pltpu.make_async_copy(o_buf.at[idx], o_hbm.at[idx], write_sem).start()

    def write_round(t, carry=None):
        for lo in write_edges[:-1]:
            write(pl.multiple_of(lo + t * _RUN, _TILE), _RUN)
        return carry

    def compute(step):
        unit = unit_of(step)
        fine_px = pl.ds(pl.multiple_of(unit * fine, fine), fine)
        coarse_px = pl.ds(pl.multiple_of(unit * coarse, coarse), coarse)
        top = jnp.dot(p_buf[:, coarse_px].reshape(_HALVES * coarse, ch), wo_buf[...],
                      preferred_element_type=jnp.float32)
        top = _upsample_rows(top).reshape(_HALVES, 1, width, ch)
        for h in range(_HALVES):
            lat = jnp.dot(c_buf[h, fine_px], wf_buf[...], preferred_element_type=jnp.float32)
            merged = lat.reshape(2, width, ch) + top[h]
            o_buf[h, fine_px] = merged.astype(o_buf.dtype).reshape(fine, ch)

    def read_phase(read_sem):
        def read(src, dst, start, size, k):
            idx = (slice(None), pl.ds(start, size))
            return pltpu.make_async_copy(src.at[idx], dst.at[idx], read_sem.at[k])

        last = len(_READ_GROUPS) - 1
        groups = [[] for _ in _READ_GROUPS]
        groups[0] += [
            pltpu.make_async_copy(wl_hbm, wl_buf, read_sem.at[0]),
            pltpu.make_async_copy(wo_hbm, wo_buf, read_sem.at[0]),
        ]
        for k, group in enumerate(groups):
            for s in range(_STREAMS):
                lo = unit_edges[s] + _READ_GROUPS[k]
                hi = unit_edges[s] + _READ_GROUPS[k + 1] if k < last else unit_edges[s + 1]
                held_back = _READ_TAIL if hi == steps else 0
                group.append(read(p_hbm, p_buf, lo * coarse, (hi - lo) * coarse, k))
                group.append(read(c_hbm, c_buf, lo * fine, (hi - lo) * fine - held_back, k))
        tail = read(c_hbm, c_buf, pixels - _READ_TAIL, _READ_TAIL, last + 1)

        def wait(group):
            for copy in group:
                copy.wait()

        for group in groups:
            for copy in group:
                copy.start()
        tail.start()

        wait(groups[0])
        wf_buf[...] = jnp.dot(
            wl_buf[...], wo_buf[...], preferred_element_type=jnp.float32
        ).astype(wf_buf.dtype)

        def read_step(step, carry):
            for k in range(1, last):
                pl.when(step == _STREAMS * _READ_GROUPS[k])(
                    functools.partial(wait, groups[k]))
            compute(step)
            return carry

        lax.fori_loop(0, _SWITCH_STEP, read_step, None)
        wait(groups[last])
        lax.fori_loop(0, _ROUNDS_AT_SWITCH, write_round, None)
        tail.wait()

    pl.run_scoped(read_phase, pltpu.SemaphoreType.DMA((len(_READ_GROUPS) + 1,)))

    def write_step(step, carry):
        for t in range(_ROUNDS_PER_STEP):
            write_round(rounds_queued(step) + t)
        compute(step)
        return carry

    lax.fori_loop(_SWITCH_STEP, steps, write_step, None)
    lax.fori_loop(rounds_queued(steps), rounds, write_round, None)
    for lo, hi in zip(write_edges[:-1], write_edges[1:]):
        if lo + rounds * _RUN < hi:
            write(lo + rounds * _RUN, hi - lo - rounds * _RUN)
    pltpu.make_async_copy(o_buf, o_hbm, write_sem).wait()


@jax.jit
def pallas_standalone__detection_seg_fpn_lateral__vision_kernel(
    c_fine: jax.Array,
    p_coarse: jax.Array,
    w_lat: jax.Array,
    w_out: jax.Array,
):
    batch, height, width, ch = c_fine.shape
    dtype = c_fine.dtype
    pixels = batch * height * width // _HALVES
    fine_shape = (_HALVES, pixels, ch)
    coarse_shape = (_HALVES, pixels // 4, ch)

    out = pl.pallas_call(
        functools.partial(_fpn_kernel, width=width),
        in_specs=[pl.BlockSpec(memory_space=pltpu.HBM)] * 4,
        out_specs=pl.BlockSpec(memory_space=pltpu.HBM),
        out_shape=jax.ShapeDtypeStruct(fine_shape, dtype),
        scratch_shapes=[
            pltpu.VMEM(fine_shape, dtype),
            pltpu.VMEM(coarse_shape, dtype),
            pltpu.VMEM(fine_shape, dtype),
            pltpu.VMEM((ch, ch), dtype),
            pltpu.VMEM((ch, ch), dtype),
            pltpu.VMEM((ch, ch), dtype),
            pltpu.SemaphoreType.DMA(()),
        ],
        compiler_params=pltpu.CompilerParams(vmem_limit_bytes=120 * 2**20),
    )(
        c_fine.reshape(fine_shape),
        p_coarse.reshape(coarse_shape),
        w_lat,
        w_out.reshape(ch, ch),
    )
    return out.reshape(batch, height, width, ch)
```
